```python
import jax
import jax.numpy as jnp

def _softmax(x, axis=-1):
    return jax.nn.softmax(x, axis=axis)
def _gelu(x):
    return jax.nn.gelu(x, approximate=True)
def _silu(x):
    return jax.nn.silu(x)
def _sigmoid(x):
    return jax.nn.sigmoid(x)
def _layernorm(x, axis=-1, eps=1e-5):
    m = jnp.mean(x, axis=axis, keepdims=True)
    v = jnp.var(x, axis=axis, keepdims=True)
    return (x - m) / jnp.sqrt(v + eps)
def _scatter_add(tgt, idx, src, axis=0):
    return tgt.at[idx].add(src)
def _segment_sum(src, seg, n):
    return jax.ops.segment_sum(src, seg, n)
class _Rng:
    def __init__(self, key):
        self._k = key
    def _next(self):
        self._k, sub = jax.random.split(self._k)
        return sub
    def normal(self, shape):
        return jax.random.normal(self._next(), shape, dtype=jnp.bfloat16)
    def randint(self, lo, hi, shape):
        return jax.random.randint(self._next(), shape, lo, hi, dtype=jnp.int32)
    def uniform(self, shape, lo=0.0, hi=1.0):
        return jax.random.uniform(self._next(), shape, jnp.bfloat16, lo, hi)
    def permutation(self, n):
        return jax.random.permutation(self._next(), n)


kernel_name = 'sequential_preLN__spectral_gfnet__swiglu_ffn__prompt'

def _fwd_setup_inputs():
    _rng = _Rng(jax.random.key(int.from_bytes(__import__("os").urandom(4), "little")))
    _w = (lambda a: (lambda t: t.astype(jnp.bfloat16) if jnp.issubdtype(t.dtype, jnp.floating) else t)(jnp.asarray(a)))
    def _A_setup():
        B, S, D = 1, 2048, 576
        Df = D // 2 + 1
        return {
            "x": _w((lambda *s: _rng.normal(s) * 0.05)(B, S, D)),
            "w_r": _w((lambda *s: _rng.normal(s) * 0.05)(S, Df) * 0.02),
            "w_i": _w((lambda *s: _rng.normal(s) * 0.05)(S, Df) * 0.02),
        }
    _A_in = _A_setup()

    def _B_setup():
        B, S, D, F = 1, 2048, 576, 4608
        return {
            "x": _w((lambda *s: _rng.normal(s) * 0.05)(B, S, D)),
            "w_gate": _w((lambda *s: _rng.normal(s) * 0.05)(D, F)),
            "w_up": _w((lambda *s: _rng.normal(s) * 0.05)(D, F)),
            "w_down": _w((lambda *s: _rng.normal(s) * 0.05)(F, D)),
        }
    _B_in = _B_setup()

    return {
        "A_x": _A_in["x"],
        "A_w_r": _A_in["w_r"],
        "A_w_i": _A_in["w_i"],
        "B_x": _B_in["x"],
        "B_w_gate": _B_in["w_gate"],
        "B_w_up": _B_in["w_up"],
        "B_w_down": _B_in["w_down"],
    }

def _fwd_reference(A_x, A_w_r, A_w_i, B_x, B_w_gate, B_w_up, B_w_down):
    def _A_ref(x, w_r, w_i):
        B, S, D = x.shape
        X = (lambda x, axes=(-2,-1): jnp.fft.rfft2(x.astype(jnp.float32), axes=axes))(x, axes=(-2, -1))
        W = w_r + 1j * w_i
        X = X * W
        y = (lambda x, s, axes=(-2,-1): jnp.fft.irfft2(x, s=s, axes=axes).astype(jnp.bfloat16))(X, (S, D), axes=(-2, -1))
        return y

    def _B_ref(x, w_gate, w_up, w_down):
        g = _silu(x @ w_gate)
        u = x @ w_up
        return (g * u) @ w_down

    x = A_x
    h = x + _A_ref(_layernorm(x, axis=-1), A_w_r, A_w_i)
    h2 = h + _B_ref(_layernorm(h, axis=-1), B_w_gate, B_w_up, B_w_down)
    return h2


def setup_inputs():
    _inp = _fwd_setup_inputs()
    _gk = jax.random.fold_in(jax.random.key(int.from_bytes(__import__("os").urandom(4), "little")), 2**31 - 1)
    _shapes = [[1, 2048, 576]]
    _dtypes = ['bfloat16']
    _gks = jax.random.split(_gk, len(_shapes))
    _gs = [jax.random.normal(k, s, dtype=jnp.dtype(d)) * 0.05 for k, s, d in zip(_gks, _shapes, _dtypes)]
    _inp["grad_out"] = _gs[0]
    return _inp

def reference(A_x, A_w_r, A_w_i, B_w_gate, B_w_up, B_w_down, B_x, grad_out):
    _const = dict(B_x=B_x)
    def _f(*_d):
        return _fwd_reference(**{'A_x': _d[0], 'A_w_r': _d[1], 'A_w_i': _d[2], 'B_w_gate': _d[3], 'B_w_up': _d[4], 'B_w_down': _d[5], **_const})
    _out, _vjp = jax.vjp(_f, A_x, A_w_r, A_w_i, B_w_gate, B_w_up, B_w_down)
    _grads = _vjp(grad_out)
    _out0 = jnp.asarray(_out)
    return (_out0, *[jnp.asarray(_g) for _g in _grads])
```

```python
import numpy as np
import jax
import jax.numpy as jnp
from jax import lax
import jax.experimental.pallas as pl
import jax.experimental.pallas.tpu as pltpu

S, D, F = 2048, 576, 4608
DF = D // 2 + 1
FP = 296
NG = FP // 8
ZR = 2 * FP
FT = 256
NF = F // FT
EPS = 1e-5
BF, F32 = jnp.bfloat16, jnp.float32


def _constants():
    f = np.arange(FP)[:, None].astype(np.float64)
    n = np.arange(D)[None, :].astype(np.float64)
    ang = 2.0 * np.pi * ((f * n) % D) / D
    live = (f < DF).astype(np.float64)
    c = (np.cos(ang) * live).reshape(NG, 1, 8, D)
    s = (-np.sin(ang) * live).reshape(NG, 1, 8, D)
    fm = np.concatenate([c, s], axis=1).reshape(ZR, D)
    a = np.arange(128)[:, None]
    lane = np.arange(128)[None, :]
    m = np.zeros((16, 256, 128), np.float64)
    for d in range(16):
        t = (d - lane) % 16
        k = 128 * t + (lane + t) % 128
        ph = 2.0 * np.pi * ((a * k) % S) / S
        m[d, :128] = np.cos(ph)
        m[d, 128:] = -np.sin(ph)
    return (fm.astype(np.float32).astype(BF), np.ascontiguousarray(fm.T).astype(np.float32).astype(BF),
            m.astype(np.float32).astype(BF))


_FM, _FMT, _MM = _constants()


def _nn(a, b):
    return jnp.dot(a, b, preferred_element_type=F32)


def _nt(a, b):
    return lax.dot_general(a, b, (((1,), (1,)), ((), ())), preferred_element_type=F32)


def _tw(xr, xi, k, sign):
    k = (k * sign) % 16
    if k == 0:
        return xr, xi
    if k == 4:
        return -xi, xr
    if k == 8:
        return -xr, -xi
    if k == 12:
        return xi, -xr
    c, s = float(np.cos(np.pi * k / 8)), float(np.sin(np.pi * k / 8))
    if k % 2 == 0:
        if c * s > 0:
            return (xr - xi) * c, (xr + xi) * c
        return (xr + xi) * c, (xi - xr) * c
    return xr * c - xi * s, xr * s + xi * c


def _dft4(r, i, sign):
    ar, ai = r[0] + r[2], i[0] + i[2]
    br, bi = r[0] - r[2], i[0] - i[2]
    cr, ci = r[1] + r[3], i[1] + i[3]
    dr, di = r[1] - r[3], i[1] - i[3]
    p = (br + di, bi - dr)
    q = (br - di, bi + dr)
    o1, o3 = (p, q) if sign < 0 else (q, p)
    return [ar + cr, o1[0], ar - cr, o3[0]], [ai + ci, o1[1], ai - ci, o3[1]]


def _dft16(r, i, sign):
    tr = [[None] * 4 for _ in range(4)]
    ti = [[None] * 4 for _ in range(4)]
    for b0 in range(4):
        yr, yi = _dft4(r[b0::4], i[b0::4], sign)
        for d0 in range(4):
            tr[d0][b0], ti[d0][b0] = _tw(yr[d0], yi[d0], b0 * d0, sign)
    outr, outi = [None] * 16, [None] * 16
    for d0 in range(4):
        yr, yi = _dft4(tr[d0], ti[d0], sign)
        for d1 in range(4):
            outr[d0 + 4 * d1], outi[d0 + 4 * d1] = yr[d1], yi[d1]
    return outr, outi


def _tile(t):
    return slice(128 * t, 128 * (t + 1))


def _radix16(z_ref, v_ref, sign):
    def body(g, carry):
        r0 = pl.multiple_of(g * 16, 16)
        r1 = pl.multiple_of(g * 16 + 8, 8)
        re = [z_ref[pl.ds(r0, 8), _tile(b)] for b in range(16)]
        im = [z_ref[pl.ds(r1, 8), _tile(b)] for b in range(16)]
        orr, oi = _dft16(re, im, sign)
        for d in range(16):
            v_ref[pl.ds(r0, 16), _tile(d)] = jnp.concatenate([orr[d], oi[d]], axis=0).astype(BF)
        return carry
    lax.fori_loop(0, NG, body, 0)


def _barrel(a, sign):
    lane = lax.broadcasted_iota(jnp.int32, a[0].shape, 1)
    for j in range(4):
        bit = (lane & (1 << j)) != 0
        a = [jnp.where(bit, a[(t + sign * (1 << j)) % 16], a[t]) for t in range(16)]
    return a


def _scale_rows(row0, nrows):
    f = row0 + lax.broadcasted_iota(jnp.int32, (nrows, 128), 0)
    return jnp.where((f == 0) | (f == DF - 1), 1.0 / (S * D), 2.0 / (S * D)).astype(F32)


def _permute_w(w_ref, wp_ref):
    def group(tiles, r0):
        a = [pltpu.bitcast(x, jnp.uint32) for x in tiles]
        a = [a[0]] + [pltpu.roll(a[t], 128 - t, 1) for t in range(1, 16)]
        a = _barrel(a, -1)
        sc = _scale_rows(r0, 16)
        for d in range(16):
            wp_ref[pl.ds(r0, 16), _tile(d)] = pltpu.bitcast(a[d], BF).astype(F32) * sc

    def body(g, carry):
        r0 = pl.multiple_of(g * 16, 16)
        group([w_ref[pl.ds(r0, 16), _tile(t)] for t in range(16)], r0)
        return carry
    lax.fori_loop(0, 18, body, 0)
    row = lax.broadcasted_iota(jnp.int32, (16, 128), 0)
    last = w_ref[288:289, :].astype(F32)
    group([jnp.where(row == 0, jnp.broadcast_to(last[:, _tile(t)], (16, 128)), 0.0).astype(BF)
           for t in range(16)], 288)


def _unpermute_dw(dwp_ref, o_ref):
    def group(r0):
        sc = _scale_rows(r0, 16)
        a = [pltpu.bitcast((dwp_ref[pl.ds(r0, 16), _tile(d)] * sc).astype(BF), jnp.uint32) for d in range(16)]
        a = _barrel(a, 1)
        a = [a[0]] + [pltpu.roll(a[t], t, 1) for t in range(1, 16)]
        return [pltpu.bitcast(x, BF) for x in a]

    def body(g, carry):
        r0 = pl.multiple_of(g * 16, 16)
        a = group(r0)
        for t in range(16):
            o_ref[pl.ds(r0, 16), _tile(t)] = a[t]
        return carry
    lax.fori_loop(0, 18, body, 0)
    a = group(288)
    for t in range(16):
        o_ref[288:289, _tile(t)] = a[t].astype(F32)[0:1, :].astype(BF)


def _split(p):
    p = p.reshape(NG, 2, 8, 256)
    return (p[:, 0, :, :128].reshape(FP, 128), p[:, 0, :, 128:].reshape(FP, 128),
            p[:, 1, :, :128].reshape(FP, 128), p[:, 1, :, 128:].reshape(FP, 128))


def _inter(re, im):
    return jnp.concatenate([re.reshape(NG, 1, 8, 128), im.reshape(NG, 1, 8, 128)], axis=1).reshape(ZR, 128)


def _fwd128(v, m):
    rr, ri, ir, ii = _split(_nn(v, jnp.concatenate([m[:128], m[128:]], axis=1)))
    return rr - ii, ri + ir


def _inv128(yr, yi, m):
    rr, ri, ir, ii = _split(_nt(_inter(yr, yi).astype(BF), m))
    return _inter(rr + ii, ir - ri)


def _ln(x):
    mu = jnp.mean(x, axis=0, keepdims=True)
    xc = x - mu
    rstd = lax.rsqrt(jnp.mean(xc * xc, axis=0, keepdims=True) + EPS)
    return xc * rstd, rstd


def _ln_bwd(dn, n, rstd):
    return rstd * (dn - jnp.mean(dn, axis=0, keepdims=True) - n * jnp.mean(dn * n, axis=0, keepdims=True))


CH = 256
NCH = S // CH


def _kernel(x_h, wr_h, wi_h, wg_h, wu_h, wd_h, do_h, fm_h, fmt_h, mm_h,
            out_h, dx_h, dwr_h, dwi_h, dwg_h, dwu_h, dwd_h,
            x_v, dot_v, wr_v, wi_v, fm_v, fmt_v, mm_v, w_v, dw_v,
            n1_v, n2t_v, n2_v, do_v, r_v, z_v, v_v, xr_v, xi_v, wpr_v, wpi_v, acc_v, dn_v,
            sem, wsem, osem):
    def lanes(c):
        return pl.ds(pl.multiple_of(c * CH, CH), CH)

    def w_in(j, slot):
        cols = pl.ds(pl.multiple_of(j * FT, FT), FT)
        return [pltpu.make_async_copy(src.at[:, cols], w_v.at[slot, k], wsem.at[slot, k])
                for k, src in enumerate((wg_h, wu_h, wd_h))]

    def w_out(j, slot):
        cols = pl.ds(pl.multiple_of(j * FT, FT), FT)
        return [pltpu.make_async_copy(dw_v.at[slot, k], dst.at[:, cols], osem.at[slot, k])
                for k, dst in enumerate((dwg_h, dwu_h, dwd_h))]

    loads = [pltpu.make_async_copy(s, d, sem.at[k]) for k, (s, d) in enumerate(
        ((x_h, x_v), (fm_h, fm_v), (wr_h, wr_v), (wi_h, wi_v), (mm_h, mm_v), (fmt_h, fmt_v), (do_h, dot_v)))]
    loads[0].start()
    loads[1].start()
    loads[0].wait()
    for c in loads[2:]:
        c.start()
    for c in w_in(0, 0):
        c.start()
    loads[1].wait()

    def p0(c, carry):
        n1, rstd = _ln(x_v[:, lanes(c)].astype(F32))
        n1 = n1.astype(BF)
        n1_v[:, lanes(c)] = n1
        r_v[0:1, lanes(c)] = rstd
        z_v[:, lanes(c)] = _nn(fm_v[...], n1)
        return carry
    lax.fori_loop(0, NCH, p0, 0)
    _radix16(z_v, v_v, -1)
    loads[2].wait()
    loads[3].wait()
    _permute_w(wr_v, wpr_v)
    _permute_w(wi_v, wpi_v)
    loads[4].wait()

    def p1(d, carry):
        t = pl.ds(pl.multiple_of(d * 128, 128), 128)
        m = mm_v[d]
        xr, xi = _fwd128(v_v[:, t], m)
        xr_v[:, t] = xr
        xi_v[:, t] = xi
        wr, wi = wpr_v[0:FP, t], wpi_v[0:FP, t]
        z_v[:, t] = _inv128(xr * wr - xi * wi, xr * wi + xi * wr, m)
        return carry
    lax.fori_loop(0, 16, p1, 0, unroll=2)
    _radix16(z_v, v_v, 1)
    loads[5].wait()
    loads[6].wait()

    def p2(c, carry):
        h = x_v[:, lanes(c)].astype(F32) + _nn(fmt_v[...], v_v[:, lanes(c)])
        acc_v[:, lanes(c)] = h
        n2, rstd = _ln(h)
        n2t_v[:, lanes(c)] = n2.astype(BF)
        r_v[1:2, lanes(c)] = rstd
        n2_v[lanes(c), :] = n2.T.astype(BF)
        do_v[lanes(c), :] = dot_v[:, lanes(c)].astype(F32).T.astype(BF)
        dn_v[:, lanes(c)] = jnp.zeros((D, CH), F32)
        return carry
    lax.fori_loop(0, NCH, p2, 0)

    def ffn(j, carry):
        slot = j % 2

        @pl.when(j + 1 < NF)
        def _():
            for c in w_in(j + 1, 1 - slot):
                c.start()
        for c in w_in(j, slot):
            c.wait()

        @pl.when(j >= 2)
        def _():
            for c in w_out(j - 2, slot):
                c.wait()
        wg, wu, wd = w_v[slot, 0], w_v[slot, 1], w_v[slot, 2]
        g = _nn(n2_v[...], wg)
        u = _nn(n2_v[...], wu)
        da = _nn(do_v[...], wd)
        sg = 0.5 * jnp.tanh(0.5 * g) + 0.5
        sl = g * sg
        a = (sl * u).astype(BF)
        du = (da * sl).astype(BF)
        dg = (da * u * (sg + sl * (1.0 - sg))).astype(BF)
        acc_v[...] += _nt(wd, a)
        dn_v[...] += _nt(wg, dg) + _nt(wu, du)
        dw_v[slot, 0] = _nn(n2t_v[...], dg).astype(BF)
        dw_v[slot, 1] = _nn(n2t_v[...], du).astype(BF)
        dw_v[slot, 2] = _nn(dot_v[...], a).astype(BF)
        for c in w_out(j, slot):
            c.start()
        return carry
    lax.fori_loop(0, NF, ffn, 0)

    def p3(c, carry):
        x_v[:, lanes(c)] = acc_v[:, lanes(c)].astype(BF)
        dh = dot_v[:, lanes(c)].astype(F32) + _ln_bwd(
            dn_v[:, lanes(c)], n2t_v[:, lanes(c)].astype(F32), r_v[1:2, lanes(c)])
        dn_v[:, lanes(c)] = dh
        z_v[:, lanes(c)] = _nn(fm_v[...], dh.astype(BF))
        return carry
    lax.fori_loop(0, NCH, p3, 0)
    out_cp = pltpu.make_async_copy(x_v, out_h, sem.at[0])
    out_cp.start()
    _radix16(z_v, v_v, -1)

    def p4(d, carry):
        t = pl.ds(pl.multiple_of(d * 128, 128), 128)
        m = mm_v[d]
        gr, gi = _fwd128(v_v[:, t], m)
        xr, xi = xr_v[:, t], xi_v[:, t]
        wr, wi = wpr_v[0:FP, t], wpi_v[0:FP, t]
        z_v[:, t] = _inv128(gr * wr + gi * wi, gi * wr - gr * wi, m)
        wpr_v[0:FP, t] = gr * xr + gi * xi
        wpi_v[0:FP, t] = gi * xr - gr * xi
        return carry
    lax.fori_loop(0, 16, p4, 0, unroll=2)
    _unpermute_dw(wpr_v, wr_v)
    _unpermute_dw(wpi_v, wi_v)
    dwr_cp = pltpu.make_async_copy(wr_v, dwr_h, sem.at[2])
    dwi_cp = pltpu.make_async_copy(wi_v, dwi_h, sem.at[3])
    dwr_cp.start()
    dwi_cp.start()
    _radix16(z_v, v_v, 1)

    def dx_cp(c):
        return pltpu.make_async_copy(n2t_v.at[:, lanes(c)], dx_h.at[:, lanes(c)], sem.at[8 + c])

    def p5(c, carry):
        dn1 = _nn(fmt_v[...], v_v[:, lanes(c)])
        dx = dn_v[:, lanes(c)] + _ln_bwd(dn1, n1_v[:, lanes(c)].astype(F32), r_v[0:1, lanes(c)])
        n2t_v[:, lanes(c)] = dx.astype(BF)
        dx_cp(c).start()
        return carry
    lax.fori_loop(0, NCH, p5, 0)

    for j in (NF - 2, NF - 1):
        for c in w_out(j, j % 2):
            c.wait()
    out_cp.wait()
    dwr_cp.wait()
    dwi_cp.wait()
    for c in range(NCH):
        dx_cp(c).wait()


@jax.jit
def pallas_sequential_preLN__spectral_gfnet__swiglu_ffn__prompt_kernel(
    A_x: jax.Array,
    A_w_r: jax.Array,
    A_w_i: jax.Array,
    B_x: jax.Array,
    B_w_gate: jax.Array,
    B_w_up: jax.Array,
    B_w_down: jax.Array,
    grad_out: jax.Array,
):
    del B_x
    hbm = pl.BlockSpec(memory_space=pltpu.HBM)
    sd = jax.ShapeDtypeStruct
    vm = pltpu.VMEM
    out, dx, dwr, dwi, dwg, dwu, dwd = pl.pallas_call(
        _kernel,
        in_specs=[hbm] * 10,
        out_specs=[hbm] * 7,
        out_shape=[sd((D, S), BF), sd((D, S), BF), sd((DF, S), BF), sd((DF, S), BF),
                   sd((D, F), BF), sd((D, F), BF), sd((D, F), BF)],
        scratch_shapes=[
            vm((D, S), BF), vm((D, S), BF), vm((DF, S), BF), vm((DF, S), BF),
            vm((ZR, D), BF), vm((D, ZR), BF), vm((16, 256, 128), BF),
            vm((2, 3, D, FT), BF), vm((2, 3, D, FT), BF),
            vm((D, S), BF), vm((D, S), BF), vm((S, D), BF), vm((S, D), BF), vm((8, S), F32),
            vm((ZR, S), F32), vm((ZR, S), BF), vm((FP, S), F32), vm((FP, S), F32),
            vm((304, S), F32), vm((304, S), F32), vm((D, S), F32), vm((D, S), F32),
            pltpu.SemaphoreType.DMA((16,)), pltpu.SemaphoreType.DMA((2, 3)), pltpu.SemaphoreType.DMA((2, 3)),
        ],
        compiler_params=pltpu.CompilerParams(vmem_limit_bytes=110 * 2**20),
    )(A_x.reshape(S, D).T, A_w_r.T, A_w_i.T, B_w_gate, B_w_up, B_w_down.T, grad_out.reshape(S, D).T,
      _FM, _FMT, _MM)
    return (out.T.reshape(1, S, D), dx.T.reshape(1, S, D), dwr.T, dwi.T, dwg, dwu, dwd.T)
```

```python
import numpy as np
import jax
import jax.numpy as jnp
from jax import lax
import jax.experimental.pallas as pl
import jax.experimental.pallas.tpu as pltpu

S, D, F = 2048, 576, 4608
DF = D // 2 + 1
FP = 296
NG = FP // 8
ZR = 2 * FP
FT = 256
NF = F // FT
EPS = 1e-5
BF, F32 = jnp.bfloat16, jnp.float32


RES = (0, 1, 3, 4, 7)
VR = 5 * 128


def _constants():
    g = np.zeros((5, 128, 128), np.float64)
    n = np.arange(64)[None, :]
    for k, e in enumerate(RES):
        if e == 0:
            f = 9 * np.arange(64)
            sig = np.ones(64)
        else:
            f = np.concatenate([e + 9 * np.arange(32), 9 - e + 9 * np.arange(32)])
            sig = np.concatenate([np.ones(32), -np.ones(32)])
        ang = 2.0 * np.pi * ((f[:, None] * n) % D) / D
        live = (f < DF)[:, None]
        c, sn, sig = np.cos(ang) * live, np.sin(ang) * live, sig[:, None]
        blk = g[k].reshape(8, 2, 8, 8, 2, 8)
        for io, ii, v in ((0, 0, c), (0, 1, sig * sn), (1, 0, -sn), (1, 1, sig * c)):
            blk[:, io, :, :, ii, :] = v.reshape(8, 8, 8, 8)
    g = np.concatenate([g, g.transpose(0, 2, 1)], axis=0)
    a = np.arange(128)[:, None]
    lane = np.arange(128)[None, :]
    m = np.zeros((16, 256, 128), np.float64)
    for d in range(16):
        t = (d - lane) % 16
        k = 128 * t + (lane + t) % 128
        ph = 2.0 * np.pi * ((a * k) % S) / S
        m[d, :128] = np.cos(ph)
        m[d, 128:] = -np.sin(ph)
    return g.astype(np.float32).astype(BF), m.astype(np.float32).astype(BF)


_GM, _MM = _constants()


def _nn(a, b):
    return jnp.dot(a, b, preferred_element_type=F32)


def _nt(a, b):
    return lax.dot_general(a, b, (((1,), (1,)), ((), ())), preferred_element_type=F32)


def _tw(xr, xi, k, sign):
    k = (k * sign) % 16
    if k == 0:
        return xr, xi
    if k == 4:
        return -xi, xr
    if k == 8:
        return -xr, -xi
    if k == 12:
        return xi, -xr
    c, s = float(np.cos(np.pi * k / 8)), float(np.sin(np.pi * k / 8))
    if k % 2 == 0:
        if c * s > 0:
            return (xr - xi) * c, (xr + xi) * c
        return (xr + xi) * c, (xi - xr) * c
    return xr * c - xi * s, xr * s + xi * c


def _dft4(r, i, sign):
    ar, ai = r[0] + r[2], i[0] + i[2]
    br, bi = r[0] - r[2], i[0] - i[2]
    cr, ci = r[1] + r[3], i[1] + i[3]
    dr, di = r[1] - r[3], i[1] - i[3]
    p = (br + di, bi - dr)
    q = (br - di, bi + dr)
    o1, o3 = (p, q) if sign < 0 else (q, p)
    return [ar + cr, o1[0], ar - cr, o3[0]], [ai + ci, o1[1], ai - ci, o3[1]]


def _dft16(r, i, sign):
    tr = [[None] * 4 for _ in range(4)]
    ti = [[None] * 4 for _ in range(4)]
    for b0 in range(4):
        yr, yi = _dft4(r[b0::4], i[b0::4], sign)
        for d0 in range(4):
            tr[d0][b0], ti[d0][b0] = _tw(yr[d0], yi[d0], b0 * d0, sign)
    outr, outi = [None] * 16, [None] * 16
    for d0 in range(4):
        yr, yi = _dft4(tr[d0], ti[d0], sign)
        for d1 in range(4):
            outr[d0 + 4 * d1], outi[d0 + 4 * d1] = yr[d1], yi[d1]
    return outr, outi


def _tile(t):
    return slice(128 * t, 128 * (t + 1))


class _Zero:
    def __add__(self, o): return o
    __radd__ = __add__
    def __sub__(self, o): return -o
    def __rsub__(self, o): return o
    def __neg__(self): return self
    def __mul__(self, o): return self


def _radix16_fwd(z_ref, v_ref):
    def body(g, carry, real):
        r0 = pl.multiple_of(g * 16, 16)
        r1 = pl.multiple_of(g * 16 + 8, 8)
        re = [z_ref[pl.ds(r0, 8), _tile(b)] for b in range(16)]
        im = [_Zero() if real else z_ref[pl.ds(r1, 8), _tile(b)] for b in range(16)]
        orr, oi = _dft16(re, im, -1)
        for d in range(16):
            i = jnp.zeros_like(orr[d]) if isinstance(oi[d], _Zero) else oi[d]
            v_ref[pl.ds(r0, 16), _tile(d)] = jnp.concatenate([orr[d], i], axis=0).astype(BF)
        return carry
    lax.fori_loop(0, 8, lambda g, c: body(g, c, True), 0, unroll=2)
    lax.fori_loop(8, 40, lambda g, c: body(g, c, False), 0, unroll=2)


def _radix16_inv(z_ref, u_ref):
    def body(g, carry, real):
        r0 = pl.multiple_of(g * 16, 16)
        r1 = pl.multiple_of(g * 16 + 8, 8)
        re = [z_ref[pl.ds(r0, 8), _tile(b)] for b in range(16)]
        im = [z_ref[pl.ds(r1, 8), _tile(b)] for b in range(16)]
        orr, oi = _dft16(re, im, 1)
        for d in range(16):
            u_ref[pl.ds(r0, 8), _tile(d)] = orr[d]
            if not real:
                u_ref[pl.ds(r1, 8), _tile(d)] = oi[d]
        return carry
    lax.fori_loop(0, 8, lambda g, c: body(g, c, True), 0, unroll=2)
    lax.fori_loop(8, 40, lambda g, c: body(g, c, False), 0, unroll=2)


_R3 = float(np.sqrt(0.75))


def _rot(xr, xi, ang):
    c, s = float(np.cos(ang)), float(np.sin(ang))
    return xr * c - xi * s, xr * s + xi * c


def _dft3(r, i, sign):
    sr, si = r[1] + r[2], i[1] + i[2]
    tr, ti = (r[1] - r[2]) * (sign * _R3), (i[1] - i[2]) * (sign * _R3)
    mr, mi = r[0] - 0.5 * sr, i[0] - 0.5 * si
    return [r[0] + sr, mr - ti, mr + ti], [i[0] + si, mi + tr, mi - tr]


def _rows(j, g):
    return slice(64 * j + 16 * g, 64 * j + 16 * g + 16)


def _radix9_fwd(get, z_ref, t):
    def r3(a, b, c):
        s = b + c
        return a + s, a - 0.5 * s, (c - b) * _R3
    for g in range(4):
        v = [get(_rows(j, g)) for j in range(9)]
        a, br, bi = zip(*[r3(v[i], v[i + 3], v[i + 6]) for i in range(3)])
        v0, v3r, v3i = r3(*a)
        c1, c2 = _rot(br[1], bi[1], -2 * np.pi / 9), _rot(br[2], bi[2], -4 * np.pi / 9)
        o_r, o_i = _dft3([br[0], c1[0], c2[0]], [bi[0], c1[1], c2[1]], -1)
        for k, pair in enumerate(((v0,), (o_r[0], o_i[0]), (v3r, v3i), (o_r[1], o_i[1]), (o_r[2], o_i[2]))):
            for im, val in enumerate(pair):
                for hh in range(2):
                    r = 128 * k + 32 * g + 16 * hh + 8 * im
                    z_ref[r:r + 8, t] = val[8 * hh:8 * hh + 8]


def _radix9_inv(z_ref, t, put):
    def r3(a, br, bi):
        m, w = a - 0.5 * br, bi * _R3
        return a + br, m - w, m + w

    def ld(r):
        return jnp.concatenate([z_ref[r:r + 8, t], z_ref[r + 16:r + 24, t]], axis=0)
    for g in range(4):
        re = [ld(128 * k + 32 * g) for k in range(5)]
        im = [None] + [ld(128 * k + 32 * g + 8) for k in range(1, 5)]
        a = r3(re[0], re[2], im[2])
        cr, ci = _dft3([re[1], re[3], re[4]], [im[1], im[3], im[4]], 1)
        b = [(cr[0], ci[0]), _rot(cr[1], ci[1], 2 * np.pi / 9), _rot(cr[2], ci[2], 4 * np.pi / 9)]
        for i in range(3):
            for k, val in enumerate(r3(a[i], *b[i])):
                put(_rows(i + 3 * k, g), val)


class _Mean:
    def __init__(self):
        self.s = None

    def add(self, v):
        self.s = v if self.s is None else self.s + v

    def get(self):
        return jnp.sum(self.s, axis=0, keepdims=True) * (1.0 / D)


_ALL = [slice(16 * i, 16 * i + 16) for i in range(D // 16)]


def _rstd(ref, t, mu):
    var = _Mean()
    for r in _ALL:
        xc = ref[r, t].astype(F32) - mu
        var.add(xc * xc)
    return lax.rsqrt(var.get() + EPS)


def _barrel(a, sign):
    lane = lax.broadcasted_iota(jnp.int32, a[0].shape, 1)
    for j in range(4):
        bit = (lane & (1 << j)) != 0
        a = [jnp.where(bit, a[(t + sign * (1 << j)) % 16], a[t]) for t in range(16)]
    return a


def _scale_rows(row0, nrows):
    f = row0 + lax.broadcasted_iota(jnp.int32, (nrows, 128), 0)
    return jnp.where((f == 0) | (f == DF - 1), 1.0 / (S * D), 2.0 / (S * D)).astype(F32)


def _permute_w(w_ref, wp_ref):
    def group(tiles, r0):
        a = [pltpu.bitcast(x, jnp.uint32) for x in tiles]
        a = [a[0]] + [pltpu.roll(a[t], 128 - t, 1) for t in range(1, 16)]
        a = _barrel(a, -1)
        sc = _scale_rows(r0, 16)
        for d in range(16):
            wp_ref[d, pl.ds(r0, 16), :] = pltpu.bitcast(a[d], BF).astype(F32) * sc

    def body(g, carry):
        r0 = pl.multiple_of(g * 16, 16)
        group([w_ref[pl.ds(r0, 16), _tile(t)] for t in range(16)], r0)
        return carry
    lax.fori_loop(0, 18, body, 0, unroll=6)
    row = lax.broadcasted_iota(jnp.int32, (16, 128), 0)
    last = w_ref[288:289, :].astype(F32)
    group([jnp.where(row == 0, jnp.broadcast_to(last[:, _tile(t)], (16, 128)), 0.0).astype(BF)
           for t in range(16)], 288)


def _unpermute_dw(dwp_ref, o_ref, side):
    def group(r0):
        sc = _scale_rows(r0, 16)
        a = [pltpu.bitcast((dwp_ref[d, pl.ds(r0, 16), :] * sc).astype(BF), jnp.uint32) for d in range(16)]
        a = _barrel(a, 1)
        a = [a[0]] + [pltpu.roll(a[t], t, 1) for t in range(1, 16)]
        return [pltpu.bitcast(x, BF) for x in a]

    side()
    for r0 in range(0, 288, 16):
        a = group(r0)
        for t in range(16):
            o_ref[r0:r0 + 16, _tile(t)] = a[t]
    a = group(288)
    for t in range(16):
        o_ref[288:289, _tile(t)] = a[t].astype(F32)[0:1, :].astype(BF)


def _cmul(dot, re, im, mr, mi, sign):
    pad = [jnp.zeros((8, 128), F32)]
    p1, p2, p3 = [dot(_cat([v] + pad, 0).astype(BF), w)[:FP] for v, w in (
        (re, mr), (im, mi), (re + im, (mr.astype(F32) + sign * mi.astype(F32)).astype(BF)))]
    return (p1 - p2, p3 - p1 - p2) if sign > 0 else (p1 + p2, p3 - p1 + p2)


def _inter(re, im):
    return jnp.concatenate([re.reshape(NG, 1, 8, 128), im.reshape(NG, 1, 8, 128)], axis=1).reshape(ZR, 128)


_WROWS = [pl.ds(0, 32, stride=9), pl.ds(288, 8)] + [
    pl.ds(o, 32, stride=9) for e in RES[1:] for o in (e, 9 - e)]


def _load_w(ref, d):
    return jnp.concatenate([ref[d, r, :] for r in _WROWS], axis=0)


def _store_w(ref, d, v):
    o = 0
    for r in _WROWS:
        ref[d, r, :] = v[o:o + r.size]
        o += r.size


def _spectral_pair(ds, cross, side, v_ref, z_ref, g_ref, m_ref, mix):
    ts = [pl.ds(d * 128 if isinstance(d, int) else pl.multiple_of(d * 128, 128), 128) for d in ds]
    z = [_nn(g_ref[k, 0:(128 if k else 80), :], _cat([v_ref[_tile(k), t] for t in ts], 1)) for k in range(5)]
    us = []
    for i, d in enumerate(ds):
        o = 1 - i if cross else i
        zi = _cat([z[0][:, _tile(i)]] + [
            v for k in range(1, 5) for v in (z[k][:64, _tile(i)], z[k][64:, _tile(o)])], 0).reshape(NG, 2, 8, 128)
        us.append(_cmul(_nn, zi[:, 0].reshape(FP, 128), zi[:, 1].reshape(FP, 128), m_ref[d, :128], m_ref[d, 128:], 1))
    side()
    us = [_inter(*_cmul(_nt, *mix(d, t, *x), m_ref[d, :128], m_ref[d, 128:], -1)).astype(BF)
          for d, t, x in zip(ds, ts, us)]
    for k in range(5):
        r = max(128 * k - 48, 0)
        lo = us[::-1] if cross and k else us
        y = _nn(g_ref[5 + k], _cat([_cat([u[r:r + 64] for u in us], 1), _cat([u[r + 64:r + 128] for u in lo], 1)], 0))
        for i, t in enumerate(ts):
            z_ref[_tile(k), t] = y[:, _tile(i)]


def _spectral_phase(first, then, side, *args):
    _spectral_pair((0, 8), False, first, *args)
    then()
    lax.fori_loop(1, 8, lambda d, c: _spectral_pair((d, 16 - d), True, lambda: side(d), *args), None)


CH = 128
NCH = S // CH
H, DH = S // 2, D // 2
XQ = 256
T2, T3, T5 = 3, 180, 216


def _tick(job, v):
    try:
        job.send(v)
    except StopIteration:
        pass

_cat = jnp.concatenate


def _pair_w(w):
    p, r = w[384:448].astype(F32), w[512:576].astype(F32)
    wa = _cat([w[256:384, :128], (p[:, :128] - p[:, 128:]).astype(BF), w[448:512, :128]], 0)
    wb = _cat([w[256:384, 128:], w[448:512, 128:], (r[:, 128:] - r[:, :128]).astype(BF)], 0)
    s = w[:256].astype(F32)
    b11, b12, b21, b22 = s[:128, :128], s[:128, 128:], s[128:, :128], s[128:, 128:]
    st = (b11 + b22, b11, b12 - b22, b21 - b11, b22, b11 + b12, b21 + b22)
    return [wa, wb, _cat([w[384:448, 128:], w[512:576, :128]], 0)] + [v.astype(BF) for v in st]


def _pair_x(lo, hi, x_ref, xs_ref, t0, t1, step=lambda v: None):
    for xt, t in ((lo, t0), (hi, t1)):
        x_ref[t, :] = _cat([xt[256:512], xt[448:576], xt[384:448], xt[512:576]], 0).T.astype(BF)
    tl, th = lo[:256].T, hi[:256].T
    a11, a12, a21, a22 = tl[:, :128], tl[:, 128:], th[:, :128], th[:, 128:]
    for i, v in enumerate((a11 + a22, a21 + a22, a11, a22, a11 + a12, a21 - a11, a12 - a22)):
        xs_ref[i, t0, :] = v.astype(BF)
        step(v[-16:])


def _pair_lhs(x_ref, xs_ref, q):
    r0, r1 = pl.ds(q * H // 8, H // 8), pl.ds(H + q * H // 8, H // 8)
    x = _cat([x_ref[r0, :], x_ref[r1, :]], 0)
    return [xs_ref[i, r0, :] for i in range(7)] + [x[:, 384:512], x[:, 0:256], _cat([x[:, 0:128], x[:, 256:384]], 1)]


def _pair_dot(xs, ws):
    t = [_pair_w(w) for w in ws]
    t = [_cat(q, 1) for q in zip(*t)]
    c = _nn(xs[7], t[2])
    m = [_nn(xs[i], t[3 + i]) for i in range(7)]
    a = _nn(xs[8], t[0]) + c + _cat([m[0] + m[3] - m[4] + m[6], m[1] + m[3]], 0)
    b = _nn(xs[9], t[1]) + c + _cat([m[2] + m[4], m[0] - m[1] + m[2] + m[5]], 0)
    return [_cat([a[:, _tile(i)], b[:, _tile(i)]], 1) for i in range(len(ws))]


def _st_act(x):
    h = x.shape[0] // 2
    tl, tr, bl, br = x[:h, :128], x[:h, 128:], x[h:, :128], x[h:, 128:]
    return [v.astype(BF) for v in (tl + br, tl, tr - br, bl - tl, br, tl + tr, bl + br)]


def _st_w(w):
    w = w.astype(F32)
    a11, a12, a21, a22 = w[:DH, :128], w[:DH, 128:], w[DH:, :128], w[DH:, 128:]
    return [v.astype(BF) for v in (a11 + a22, a21 - a22, a12 + a22, a11 + a21, a12 - a11, a22, a11)]


def _st_tok(lo, hi):
    a11, a12, a21, a22 = lo[:DH], hi[:DH], lo[DH:], hi[DH:]
    return [v.astype(BF) for v in (a11 + a22, a21 + a22, a11, a22, a11 + a12, a21 - a11, a12 - a22)]


def _st_dw(o, m):
    o[:DH, :128] = (m[0] + m[3] - m[4] + m[6]).astype(BF)
    o[:DH, 128:] = (m[2] + m[4]).astype(BF)
    o[DH:, :128] = (m[1] + m[3]).astype(BF)
    o[DH:, 128:] = (m[0] - m[1] + m[2] + m[5]).astype(BF)


def _st_acc(ref, t, put):
    for r in _ALL[:DH // 16]:
        m = [ref[i, r, t] for i in range(7)]
        r2 = slice(r.start + DH, r.stop + DH)
        put(0, r, m[0] + m[4] - m[5] + m[2])
        put(0, r2, m[1] + m[5])
        put(1, r, m[6] + m[4])
        put(1, r2, m[0] - m[6] + m[1] + m[3])


def _kernel(x_h, wr_h, wi_h, wg_h, wu_h, wd_h, do_h, gm_h, mm_h,
            out_h, dx_h, dwr_h, dwi_h, dwg_h, dwu_h, dwd_h,
            x_v, dot_v, wr_v, wi_v, gm_v, mm_v, w_v, dw_v,
            n1_v, n2t_v, n2_v, do_v, n2q_v, doq_v, r_v, z_v, u_v, v_v, xr_v, xi_v, wpr_v, wpi_v, acc_v, dn_v, n2s_v, dos_v, dh_v,
            la_v, lp_v, dwd_v, dq_v, wd_v, da_v, sem, wsem, osem, xsem, dsem):
    def lanes(c):
        return pl.ds(c * CH if isinstance(c, int) else pl.multiple_of(c * CH, CH), CH)

    def w_in(j, slot):
        cols = pl.ds(pl.multiple_of(j * FT, FT), FT)
        return [pltpu.make_async_copy(src.at[:, cols], w_v.at[slot, k], wsem.at[slot, k])
                for k, src in enumerate((wg_h, wu_h))]

    def w_out(j, slot):
        cols = pl.ds(pl.multiple_of(j * FT, FT), FT)
        return [pltpu.make_async_copy(dw_v.at[slot, k], dst.at[:, cols], osem.at[slot, k])
                for k, dst in enumerate((dwg_h, dwu_h))] + [
            pltpu.make_async_copy(dq_v.at[slot, k], dwd_h.at[k * DH:(k + 1) * DH, lanes(2 * j + 1 - k)],
                                  osem.at[slot, 2 + k]) for k in range(2)]

    loads = [pltpu.make_async_copy(s, d, sem.at[k]) for k, (s, d) in enumerate(
        ((wr_h, wr_v), (wi_h, wi_v), (gm_h, gm_v), (mm_h, mm_v), (do_h, dot_v)))]

    def x_in(q):
        cols = pl.ds(q * XQ if isinstance(q, int) else pl.multiple_of(q * XQ, XQ), XQ)
        return pltpu.make_async_copy(x_h.at[:, cols], x_v.at[:, cols], xsem.at[q])
    x_in(0).start()
    x_in(1).start()
    x_in(2).start()

    def p0(q, carry):
        x_in(q).wait()

        @pl.when(q + 3 < S // XQ)
        def _():
            x_in(q + 3).start()

        @pl.when(q == 4)
        def _():
            loads[0].start()
            loads[1].start()

        @pl.when(q == 7)
        def _():
            loads[2].start()
            loads[3].start()
        for t in (lanes(2 * q), lanes(2 * q + 1)):
            mean = _Mean()
            for r in _ALL:
                mean.add(x_v[r, t].astype(F32))
            mu = mean.get()
            rstd = _rstd(x_v, t, mu)
            r_v[0:1, t] = rstd

            def get(r):
                n1 = (x_v[r, t].astype(F32) - mu) * rstd
                n1_v[r, t] = n1.astype(BF)
                return n1
            _radix9_fwd(get, z_v, t)
        return carry
    lax.fori_loop(0, S // XQ, p0, 0)
    _radix16_fwd(z_v, v_v)
    loads[4].start()
    loads[0].wait()
    _permute_w(wr_v, wpr_v)
    loads[1].wait()
    _permute_w(wi_v, wpi_v)
    loads[2].wait()
    loads[3].wait()
    wd_cp = pltpu.make_async_copy(wd_h, wd_v, sem.at[5])

    def start_ffn_loads():
        loads[4].wait()
        for cp in [wd_cp] + w_in(0, 0):
            cp.start()

    def mix_fwd(d, t, xr, xi):
        xr_v[:, t] = xr
        xi_v[:, t] = xi
        wr, wi = _load_w(wpr_v, d), _load_w(wpi_v, d)
        return xr * wr - xi * wi, xr * wi + xi * wr

    def prep_do(c):
        t = lanes(c)
        ds = []
        for tt in (t, lanes(c + NCH // 2)):
            ds.append(dot_v[:, tt].astype(F32))
        _pair_x(*ds, do_v, doq_v, t, tt)
        for i, v in enumerate(_st_tok(*ds)):
            dos_v[i, :, t] = v
    _spectral_phase(lambda: None, start_ffn_loads, lambda d: prep_do(d - 1), v_v, z_v, gm_v, mm_v, mix_fwd)
    _radix16_inv(z_v, u_v)

    wd_cp.wait()

    def early(p, ticks):
        xs = _pair_lhs(do_v, doq_v, 0)
        rows = [[x[r:r + 16] for r in range(0, x.shape[0], 16)] for x in xs]
        todo = [(x, r) for x in rows for r in range(len(x))]
        cost = np.cumsum([x[r].shape[1] for x, r in todo])
        done = 1
        for step in range(ticks):
            tok = yield
            while cost[done] * ticks <= step * cost[-1]:
                x, r = todo[done]
                x[r] = _cat([jnp.where(p < 0, tok.astype(BF), x[r][:, :128]), x[r][:, 128:]][:x[r].shape[1] // 128], 1)
                done += 1
        cols = [(2 * p + i) * FT for i in range(2)]
        ws = [wd_v[:, pl.ds(o if isinstance(o, int) else pl.multiple_of(o, FT), FT)] for o in cols]
        da_v[2 * p], da_v[2 * p + 1] = _pair_dot([_cat(x, 0) for x in rows], ws)
    list(early(NF // 2 - 1, 0))
    prep_do(NCH // 2 - 1)

    def p2(c, carry):
        job = early(c, 72 + 14 * T2)
        next(job)

        def step(v):
            for _ in range(T2):
                _tick(job, v)
        t = lanes(c)
        th = lanes(c + NCH // 2)
        ns = []
        for tt in (t, th):
            mean = _Mean()

            def put(r, y):
                h = (x_v[r, tt].astype(F32) + y).astype(BF)
                x_v[r, tt] = h
                mean.add(h.astype(F32))
                _tick(job, h)
            _radix9_inv(u_v, tt, put)
            mu = mean.get()
            rstd = _rstd(x_v, tt, mu)
            r_v[1:2, tt] = rstd
            ns.append((x_v[:, tt].astype(F32) - mu) * rstd)
            n2t_v[:, tt] = ns[-1].astype(BF)
        _pair_x(*ns, n2_v, n2q_v, t, th, step)
        for i, v in enumerate(_st_tok(*ns)):
            n2s_v[i, :, t] = v
            step(v[-16:])
        assert next(job, 0) == 0
        return carry
    lax.fori_loop(0, NCH // 2, p2, 0)

    def ffn(j, carry):
        slot = j % 2

        @pl.when(j + 1 < NF)
        def _():
            for c in w_in(j + 1, 1 - slot):
                c.start()
        for c in w_in(j, slot):
            c.wait()

        @pl.when(j >= 2)
        def _():
            for c in w_out(j - 2, slot):
                c.wait()
        wg, wu, wd = w_v[slot, 0], w_v[slot, 1], wd_v[:, pl.ds(pl.multiple_of(j * FT, FT), FT)]
        parts = []
        for q in range(8):
            da = _pair_dot(_pair_lhs(do_v, doq_v, q), [wd])[0] if q else da_v[j]
            g, u = _pair_dot(_pair_lhs(n2_v, n2q_v, q), [wg, wu])
            sg = 0.5 * jnp.tanh(0.5 * g) + 0.5
            sl = g * sg
            parts.append(_st_act(sl * u) + _st_act(da * sl) + _st_act(da * u * (sg + sl * (1.0 - sg))))
        parts = [_cat(v, 0) for v in zip(*parts)]
        ca, cu, cg = parts[:7], parts[7:14], parts[14:]
        xd, xg, xu = _st_w(wd), _st_w(wg), _st_w(wu)
        for t in (slice(0, H // 2), slice(H // 2, H)):
            for i in range(7):
                acc_v[i, :, t] = jnp.where(j > 0, acc_v[i, :, t], 0.0) + _nt(xd[i], ca[i][t])
                dn_v[i, :, t] = jnp.where(j > 0, dn_v[i, :, t], 0.0) + _nt(
                    _cat([xg[i], xu[i]], 1), _cat([cg[i][t], cu[i][t]], 1))
        mm = [_nn(n2s_v[i], _cat([cg[i], cu[i]], 1)) for i in range(7)]
        _st_dw(dw_v.at[slot, 0], [m[:, :128] for m in mm])
        _st_dw(dw_v.at[slot, 1], [m[:, 128:] for m in mm])
        pair, half = j // 2, lanes(slot)
        la_v[0, pair, :, half] = ca[6]
        la_v[1, pair, :, half] = ca[5]
        m = [_nn(dos_v[i], ca[i]) for i in range(5)]
        lp_v[0, pair, :, half] = m[0] + m[3] - m[4]
        lp_v[1, pair, :, half] = m[0] - m[1] + m[2]
        dq_v[slot, 0] = (m[2] + m[4]).astype(BF)
        dq_v[slot, 1] = (m[1] + m[3]).astype(BF)
        for c in w_out(j, slot):
            c.start()
        return carry
    lax.fori_loop(0, NF, ffn, 0)

    def late(k, p, ticks):
        todo = []
        for c in range(4):
            ks = slice(c // 2 * H // 2, (c // 2 + 1) * H // 2)
            todo.append(lambda ks=ks, c=c: la_v[k, p, ks, _tile(c % 2)])
            todo += [lambda ks=ks, r=r: dos_v[6 - k, r, ks] for r in _ALL[:DH // 16]]
        got, n = [], len(todo) // 4
        for step in range(ticks):
            tok = yield
            while len(got) < len(todo) and len(got) * ticks <= step * len(todo):
                v = todo[len(got)]()
                if len(got) % n > 1:
                    v = _cat([jnp.where(p < 0, tok.astype(BF), v[:, :128]), v[:, 128:]], 1)
                got.append(v)
        got += [f() for f in todo[len(got):]]
        m = [_nn(_cat(got[c * n + 1:(c + 1) * n], 0), got[c * n]) for c in range(4)]
        for i in range(2):
            dwd_v[k, p, i] = (lp_v[k, p, :, _tile(i)] + m[i] + m[i + 2]).astype(BF)

    def late_out(k, p):
        return [pltpu.make_async_copy(dwd_v.at[k, p, i], dwd_h.at[k * DH:(k + 1) * DH, lanes(4 * p + 2 * i + k)],
                                      dsem.at[k, p, i]) for i in range(2)]

    def p3(c, carry):
        job = late(0, c, T3)
        next(job)
        ts = (lanes(c), lanes(c + NCH // 2))
        m1, m2 = (_Mean(), _Mean()), (_Mean(), _Mean())

        def put(i, r, dn):
            _tick(job, dn)
            u_v[r, ts[i]] = dn
            m1[i].add(dn)
            m2[i].add(dn * n2t_v[r, ts[i]].astype(F32))
        _st_acc(dn_v, ts[0], put)
        for i, t in enumerate(ts):
            a, b, rstd = m1[i].get(), m2[i].get(), r_v[1:2, t]

            def get(r):
                dh = dot_v[r, t].astype(F32) + rstd * (u_v[r, t] - a - n2t_v[r, t].astype(F32) * b)
                dh_v[r, t] = dh
                _tick(job, dh)
                if r.start % 32 == 0:
                    _tick(job, dh)
                return dh
            _radix9_fwd(get, z_v, t)
        assert next(job, 0) == 0
        for cp in late_out(0, c):
            cp.start()
        return carry
    lax.fori_loop(0, NCH // 2, p3, 0)
    _radix16_fwd(z_v, v_v)

    def mix_bwd(d, t, gr, gi):
        xr, xi = xr_v[:, t], xi_v[:, t]
        wr, wi = _load_w(wpr_v, d), _load_w(wpi_v, d)
        _store_w(wpr_v, d, gr * xr + gi * xi)
        _store_w(wpi_v, d, gi * xr - gr * xi)
        return gr * wr + gi * wi, gi * wr - gr * wi

    def fin_out(c):
        ts = (lanes(c), lanes(c + NCH // 2))

        def put(i, r, o):
            x_v[r, ts[i]] = (x_v[r, ts[i]].astype(F32) + o).astype(BF)
        _st_acc(acc_v, ts[0], put)
    _spectral_phase(lambda: fin_out(0), lambda: None, fin_out, v_v, z_v, gm_v, mm_v, mix_bwd)
    out_cp = pltpu.make_async_copy(x_v, out_h, sem.at[0])
    out_cp.start()
    _unpermute_dw(wpr_v, wr_v, lambda: list(late(0, NF // 2 - 1, 0)))
    _unpermute_dw(wpi_v, wi_v, lambda: list(late(1, NF // 2 - 1, 0)))
    for cp in late_out(0, NF // 2 - 1) + late_out(1, NF // 2 - 1):
        cp.start()
    dwr_cp = pltpu.make_async_copy(wr_v, dwr_h, sem.at[2])
    dwi_cp = pltpu.make_async_copy(wi_v, dwi_h, sem.at[3])
    dwr_cp.start()
    dwi_cp.start()
    _radix16_inv(z_v, u_v)

    def dx_cp(q):
        cols = pl.ds(q * XQ if isinstance(q, int) else pl.multiple_of(q * XQ, XQ), XQ)
        return pltpu.make_async_copy(n2t_v.at[:, cols], dx_h.at[:, cols], xsem.at[q])

    def p5(q, carry):
        job = late(1, q, T5)
        next(job)
        stats = []
        for t in (lanes(2 * q), lanes(2 * q + 1)):
            m1, m2 = _Mean(), _Mean()

            def put(r, dn):
                _tick(job, dn)
                z_v[r, t] = dn
                _tick(job, dn)
                m1.add(dn)
                m2.add(dn * n1_v[r, t].astype(F32))
            _radix9_inv(u_v, t, put)
            stats.append((t, m1.get(), m2.get(), r_v[0:1, t]))
        for t, a, b, rstd in stats:
            for r in _ALL:
                dx = dh_v[r, t] + rstd * (z_v[r, t] - a - n1_v[r, t].astype(F32) * b)
                n2t_v[r, t] = dx.astype(BF)
                _tick(job, dx)
        assert next(job, 0) == 0
        dx_cp(q).start()
        for cp in late_out(1, q):
            cp.start()
        return carry
    lax.fori_loop(0, S // XQ, p5, 0)

    for j in (NF - 2, NF - 1):
        for c in w_out(j, j % 2):
            c.wait()
    out_cp.wait()
    dwr_cp.wait()
    dwi_cp.wait()
    for q in range(S // XQ):
        dx_cp(q).wait()
    for p in range(NF // 2):
        for cp in late_out(0, p) + late_out(1, p):
            cp.wait()


@jax.jit
def pallas_sequential_preLN__spectral_gfnet__swiglu_ffn__prompt_kernel(
    A_x: jax.Array,
    A_w_r: jax.Array,
    A_w_i: jax.Array,
    B_x: jax.Array,
    B_w_gate: jax.Array,
    B_w_up: jax.Array,
    B_w_down: jax.Array,
    grad_out: jax.Array,
):
    del B_x
    hbm = pl.BlockSpec(memory_space=pltpu.HBM)
    sd = jax.ShapeDtypeStruct
    vm = pltpu.VMEM
    out, dx, dwr, dwi, dwg, dwu, dwd = pl.pallas_call(
        _kernel,
        in_specs=[hbm] * 9,
        out_specs=[hbm] * 7,
        out_shape=[sd((D, S), BF), sd((D, S), BF), sd((DF, S), BF), sd((DF, S), BF),
                   sd((D, F), BF), sd((D, F), BF), sd((D, F), BF)],
        scratch_shapes=[
            vm((D, S), BF), vm((D, S), BF), vm((DF, S), BF), vm((DF, S), BF),
            vm((10, 128, 128), BF), vm((16, 256, 128), BF),
            vm((2, 2, D, FT), BF), vm((2, 2, D, FT), BF),
            vm((D, S), BF), vm((D, S), BF), vm((S, 512), BF), vm((S, 512), BF),
            vm((7, H, 128), BF), vm((7, H, 128), BF), vm((8, S), F32),
            vm((VR, S), F32), vm((VR, S), F32), vm((VR, S), BF), vm((FP, S), F32), vm((FP, S), F32),
            vm((16, 304, 128), F32), vm((16, 304, 128), F32), vm((7, DH, H), F32), vm((7, DH, H), F32),
            vm((7, DH, H), BF), vm((7, DH, H), BF), vm((D, S), F32),
            vm((2, NF // 2, H, 256), BF), vm((2, NF // 2, DH, 256), F32), vm((2, NF // 2, 2, DH, 128), BF),
            vm((2, 2, DH, 128), BF), vm((D, F), BF), vm((NF, 256, FT), F32),
            pltpu.SemaphoreType.DMA((6,)), pltpu.SemaphoreType.DMA((2, 2)), pltpu.SemaphoreType.DMA((2, 4)),
            pltpu.SemaphoreType.DMA((S // XQ,)), pltpu.SemaphoreType.DMA((2, NF // 2, 2)),
        ],
        compiler_params=pltpu.CompilerParams(vmem_limit_bytes=124 * 2**20),
    )(A_x.reshape(S, D).T, A_w_r.T, A_w_i.T, B_w_gate, B_w_up, B_w_down.T, grad_out.reshape(S, D).T,
      _GM, _MM)
    return (out.T.reshape(1, S, D), dx.T.reshape(1, S, D), dwr.T, dwi.T, dwg, dwu, dwd.T)
```
